```python
import os as _os
_os.environ.setdefault("JAX_PLATFORMS", "cpu")
import jax
import jax.numpy as jnp

def _softmax(x, axis=-1):
    return jax.nn.softmax(x, axis=axis)
def _gelu(x):
    return jax.nn.gelu(x, approximate=True)
def _silu(x):
    return jax.nn.silu(x)
def _sigmoid(x):
    return jax.nn.sigmoid(x)
def _layernorm(x, axis=-1, eps=1e-5):
    m = jnp.mean(x, axis=axis, keepdims=True)
    v = jnp.var(x, axis=axis, keepdims=True)
    return (x - m) / jnp.sqrt(v + eps)
def _scatter_add(tgt, idx, src, axis=0):
    return tgt.at[idx].add(src)
def _segment_sum(src, seg, n):
    return jax.ops.segment_sum(src, seg, n)
class _Rng:
    def __init__(self, key):
        self._k = key
    def _next(self):
        self._k, sub = jax.random.split(self._k)
        return sub
    def normal(self, shape):
        return jax.random.normal(self._next(), shape, dtype=jnp.bfloat16)
    def randint(self, lo, hi, shape):
        return jax.random.randint(self._next(), shape, lo, hi, dtype=jnp.int32)
    def uniform(self, shape, lo=0.0, hi=1.0):
        return jax.random.uniform(self._next(), shape, jnp.bfloat16, lo, hi)
    def permutation(self, n):
        return jax.random.permutation(self._next(), n)


kernel_name = 'standalone__gqa_block_cached__near_ridge'

def setup_inputs():
    _rng = _Rng(jax.random.key(int.from_bytes(__import__("os").urandom(4), "little")))
    _w = (lambda a: (lambda t: t.astype(jnp.bfloat16) if jnp.issubdtype(t.dtype, jnp.floating) else t)(jnp.asarray(a)))
    B, Sq, D = 8, 64, 512
    Hq, Hkv, Sk, Dh = 32, 8, 64, 128
    assert Hq % Hkv == 0, (Hq, Hkv)
    return {
        "x": _w((lambda *s: _rng.normal(s) * 0.8)(B, Sq, D)),
        "k_cache": _w((lambda *s: _rng.normal(s) * 0.8)(B, Hkv, Sk, Dh)),
        "v_cache": _w((lambda *s: _rng.normal(s) * 0.05)(B, Hkv, Sk, Dh)),
        "wq": _w((lambda *s: _rng.normal(s) * 0.8)(D, Hq * Dh) * (D ** -0.5)),
        "wo": _w((lambda *s: _rng.normal(s) * 0.05)(Hq * Dh, D) * ((Hq * Dh) ** -0.5)),
    }

def reference(x, k_cache, v_cache, wq, wo):
    B, Sq, D = x.shape
    Hq, Dh = 32, 128
    Hkv = k_cache.shape[1]
    rep = Hq // Hkv
    q = (lambda x, *d: x.transpose(*d))((x @ wq).reshape(B, Sq, Hq, Dh), 0, 2, 1, 3)
    k = jnp.repeat(k_cache, rep, axis=1)
    v = jnp.repeat(v_cache, rep, axis=1)
    scores = jnp.einsum("bhqd,bhkd->bhqk", q, k) * (Dh ** -0.5)
    p = _softmax(scores, axis=-1)
    o = jnp.einsum("bhqk,bhkd->bhqd", p, v)
    return (lambda x, *d: x.transpose(*d))(o, 0, 2, 1, 3).reshape(B, Sq, Hq * Dh) @ wo
```

```python
import functools

import jax
import jax.numpy as jnp
from jax import lax
import jax.experimental.pallas as pl
import jax.experimental.pallas.tpu as pltpu


@jax.jit
def pallas_standalone__gqa_block_cached__near_ridge_kernel(
    x: jax.Array,
    k_cache: jax.Array,
    v_cache: jax.Array,
    wq: jax.Array,
    wo: jax.Array,
):
    B, Sq, D = x.shape
    _, Hkv, Sk, Dh = k_cache.shape
    Hq = wq.shape[1] // Dh
    rep = Hq // Hkv
    scale = Dh ** -0.5

    def kernel(x_ref, k_ref, v_ref, wq_ref, wo_ref, o_ref, acc_ref):
        g = pl.program_id(0)

        @pl.when(g == 0)
        def _():
            acc_ref[...] = jnp.zeros_like(acc_ref)

        xm = x_ref[...].reshape(B * Sq, D)
        q = jnp.dot(xm, wq_ref[...], preferred_element_type=jnp.float32)
        q = q.astype(jnp.bfloat16)

        outs = []
        for b in range(B):
            qb = q[b * Sq:(b + 1) * Sq, :]
            qh = jnp.concatenate(
                [qb[:, h * Dh:(h + 1) * Dh] for h in range(rep)], axis=0)
            kb = k_ref[b, 0]
            vb = v_ref[b, 0]
            s = lax.dot_general(
                qh, kb, (((1,), (1,)), ((), ())),
                preferred_element_type=jnp.float32)
            s = (s.astype(jnp.bfloat16) * jnp.bfloat16(scale)).astype(jnp.float32)
            m = jnp.max(s, axis=-1, keepdims=True)
            e = jnp.exp(s - m)
            p = (e / jnp.sum(e, axis=-1, keepdims=True)).astype(jnp.bfloat16)
            ob = jnp.dot(p, vb, preferred_element_type=jnp.float32)
            ob = ob.astype(jnp.bfloat16)
            ob = jnp.concatenate(
                [ob[h * Sq:(h + 1) * Sq, :] for h in range(rep)], axis=1)
            outs.append(ob)
        o = jnp.concatenate(outs, axis=0)
        acc_ref[...] += jnp.dot(o, wo_ref[...], preferred_element_type=jnp.float32)

        @pl.when(g == pl.num_programs(0) - 1)
        def _():
            o_ref[...] = acc_ref[...].astype(o_ref.dtype).reshape(o_ref.shape)

    grid_spec = pltpu.PrefetchScalarGridSpec(
        num_scalar_prefetch=0,
        grid=(Hkv,),
        in_specs=[
            pl.BlockSpec((B, Sq, D), lambda g: (0, 0, 0)),
            pl.BlockSpec((B, 1, Sk, Dh), lambda g: (0, g, 0, 0)),
            pl.BlockSpec((B, 1, Sk, Dh), lambda g: (0, g, 0, 0)),
            pl.BlockSpec((D, rep * Dh), lambda g: (0, g)),
            pl.BlockSpec((rep * Dh, D), lambda g: (g, 0)),
        ],
        out_specs=pl.BlockSpec((B, Sq, D), lambda g: (0, 0, 0)),
        scratch_shapes=[pltpu.VMEM((B * Sq, D), jnp.float32)],
    )
    out_shape = jax.ShapeDtypeStruct((B, Sq, D), jnp.bfloat16)

    return pl.pallas_call(
        kernel,
        grid_spec=grid_spec,
        out_shape=out_shape,
        compiler_params=pltpu.CompilerParams(
            dimension_semantics=("arbitrary",),
            vmem_limit_bytes=64 * 1024 * 1024,
        ),
    )(x, k_cache, v_cache, wq, wo)
```

```python
import jax
import jax.numpy as jnp
from jax import lax
import jax.experimental.pallas as pl
import jax.experimental.pallas.tpu as pltpu


@jax.jit
def pallas_standalone__gqa_block_cached__near_ridge_kernel(
    x: jax.Array,
    k_cache: jax.Array,
    v_cache: jax.Array,
    wq: jax.Array,
    wo: jax.Array,
):
    B, Sq, D = x.shape
    _, Hkv, Sk, Dh = k_cache.shape
    Hq = wq.shape[1] // Dh
    rep = Hq // Hkv
    c = (Dh ** -0.5) * 1.4426950408889634

    def kernel(x_ref, k_ref, v_ref, wq_ref, wo_ref, o_ref, acc_ref):
        g = pl.program_id(0)

        @pl.when(g == 0)
        def _():
            acc_ref[...] = jnp.zeros_like(acc_ref)

        xm = x_ref[...].reshape(B * Sq, D)
        q = jnp.dot(xm, wq_ref[...], preferred_element_type=jnp.float32)
        q = q.astype(jnp.bfloat16)

        outs = []
        for b in range(B):
            qb = q[b * Sq:(b + 1) * Sq, :]
            qh = jnp.concatenate(
                [qb[:, h * Dh:(h + 1) * Dh] for h in range(rep)], axis=0)
            kb = k_ref[b, 0]
            vb = v_ref[b, 0]
            s = lax.dot_general(
                qh, kb, (((1,), (1,)), ((), ())), preferred_element_type=jnp.float32)
            m = jnp.max(s, axis=-1, keepdims=True)
            e = jnp.exp2((s - m) * jnp.float32(c))
            r = pl.reciprocal(jnp.sum(e, axis=-1, keepdims=True),
                              approx=False, full_range=False)
            p = (e * r).astype(jnp.bfloat16)
            ob = jnp.dot(p, vb, preferred_element_type=jnp.float32)
            ob = ob.astype(jnp.bfloat16)
            outs.append(jnp.concatenate(
                [ob[h * Sq:(h + 1) * Sq, :] for h in range(rep)], axis=1))
        o = jnp.concatenate(outs, axis=0)
        acc_ref[...] += jnp.dot(o, wo_ref[...], preferred_element_type=jnp.float32)

        @pl.when(g == pl.num_programs(0) - 1)
        def _():
            o_ref[...] = acc_ref[...].astype(o_ref.dtype).reshape(o_ref.shape)

    grid_spec = pltpu.PrefetchScalarGridSpec(
        num_scalar_prefetch=0,
        grid=(Hkv,),
        in_specs=[
            pl.BlockSpec((B, Sq, D), lambda g: (0, 0, 0)),
            pl.BlockSpec((B, 1, Sk, Dh), lambda g: (0, g, 0, 0)),
            pl.BlockSpec((B, 1, Sk, Dh), lambda g: (0, g, 0, 0)),
            pl.BlockSpec((D, rep * Dh), lambda g: (0, g)),
            pl.BlockSpec((rep * Dh, D), lambda g: (g, 0)),
        ],
        out_specs=pl.BlockSpec((B, Sq, D), lambda g: (0, 0, 0)),
        scratch_shapes=[pltpu.VMEM((B * Sq, D), jnp.float32)],
    )
    out_shape = jax.ShapeDtypeStruct((B, Sq, D), jnp.bfloat16)

    return pl.pallas_call(
        kernel,
        grid_spec=grid_spec,
        out_shape=out_shape,
        compiler_params=pltpu.CompilerParams(
            dimension_semantics=("arbitrary",),
            vmem_limit_bytes=64 * 1024 * 1024,
        ),
    )(x, k_cache, v_cache, wq, wo)
```

```python
import jax
import jax.numpy as jnp
from jax import lax
import jax.experimental.pallas as pl
import jax.experimental.pallas.tpu as pltpu


@jax.jit
def pallas_standalone__gqa_block_cached__near_ridge_kernel(
    x: jax.Array,
    k_cache: jax.Array,
    v_cache: jax.Array,
    wq: jax.Array,
    wo: jax.Array,
):
    B, Sq, D = x.shape
    _, Hkv, Sk, Dh = k_cache.shape
    Hq = wq.shape[1] // Dh
    rep = Hq // Hkv
    log2e = 1.4426950408889634

    def kernel(x_ref, k_ref, v_ref, wq_ref, wo_ref, o_ref, acc_ref):
        g = pl.program_id(0)

        @pl.when(g == 0)
        def _():
            acc_ref[...] = jnp.zeros_like(acc_ref)

        xm = x_ref[...].reshape(B * Sq, D)
        q = jnp.dot(xm, wq_ref[...], preferred_element_type=jnp.float32)
        q = q.astype(jnp.bfloat16)

        def scores_t(b):
            qb = q[b * Sq:(b + 1) * Sq, :]
            qh = jnp.concatenate(
                [qb[:, h * Dh:(h + 1) * Dh] for h in range(rep)], axis=0)
            return lax.dot_general(
                k_ref[b, 0], qh, (((1,), (1,)), ((), ())),
                preferred_element_type=jnp.float32)

        sTs = [scores_t(b) for b in range(B)]
        pTs = []
        for b in range(B):
            sT = (sTs[b].astype(jnp.bfloat16) * jnp.bfloat16(Dh ** -0.5)).astype(jnp.float32)
            m = jnp.max(sT, axis=0, keepdims=True)
            e = jnp.exp2((sT - m) * jnp.float32(log2e))
            r = pl.reciprocal(jnp.sum(e, axis=0, keepdims=True),
                              approx=False, full_range=False)
            pTs.append((e * r).astype(jnp.bfloat16))
        oTs = [jnp.dot(v_ref[b, 0].T, pTs[b], preferred_element_type=jnp.float32)
               for b in range(B)]
        outs = []
        for b in range(B):
            ob = oTs[b].astype(jnp.bfloat16).T
            outs.append(jnp.concatenate(
                [ob[h * Sq:(h + 1) * Sq, :] for h in range(rep)], axis=1))
        o = jnp.concatenate(outs, axis=0)
        acc_ref[...] += jnp.dot(o, wo_ref[...], preferred_element_type=jnp.float32)

        @pl.when(g == pl.num_programs(0) - 1)
        def _():
            o_ref[...] = acc_ref[...].astype(o_ref.dtype).reshape(o_ref.shape)

    grid_spec = pltpu.PrefetchScalarGridSpec(
        num_scalar_prefetch=0,
        grid=(Hkv,),
        in_specs=[
            pl.BlockSpec((B, Sq, D), lambda g: (0, 0, 0)),
            pl.BlockSpec((B, 1, Sk, Dh), lambda g: (0, g, 0, 0)),
            pl.BlockSpec((B, 1, Sk, Dh), lambda g: (0, g, 0, 0)),
            pl.BlockSpec((D, rep * Dh), lambda g: (0, g)),
            pl.BlockSpec((rep * Dh, D), lambda g: (g, 0)),
        ],
        out_specs=pl.BlockSpec((B, Sq, D), lambda g: (0, 0, 0)),
        scratch_shapes=[pltpu.VMEM((B * Sq, D), jnp.float32)],
    )
    out_shape = jax.ShapeDtypeStruct((B, Sq, D), jnp.bfloat16)

    return pl.pallas_call(
        kernel,
        grid_spec=grid_spec,
        out_shape=out_shape,
        compiler_params=pltpu.CompilerParams(
            dimension_semantics=("arbitrary",),
            vmem_limit_bytes=64 * 1024 * 1024,
        ),
    )(x, k_cache, v_cache, wq, wo)
```
